```python
import os as _os
_os.environ.setdefault("JAX_PLATFORMS", "cpu")
import jax
import jax.numpy as jnp

def _softmax(x, axis=-1):
    return jax.nn.softmax(x, axis=axis)
def _gelu(x):
    return jax.nn.gelu(x, approximate=True)
def _silu(x):
    return jax.nn.silu(x)
def _sigmoid(x):
    return jax.nn.sigmoid(x)
def _layernorm(x, axis=-1, eps=1e-5):
    m = jnp.mean(x, axis=axis, keepdims=True)
    v = jnp.var(x, axis=axis, keepdims=True)
    return (x - m) / jnp.sqrt(v + eps)
def _scatter_add(tgt, idx, src, axis=0):
    return tgt.at[idx].add(src)
def _segment_sum(src, seg, n):
    return jax.ops.segment_sum(src, seg, n)
class _Rng:
    def __init__(self, key):
        self._k = key
    def _next(self):
        self._k, sub = jax.random.split(self._k)
        return sub
    def normal(self, shape):
        return jax.random.normal(self._next(), shape, dtype=jnp.bfloat16)
    def randint(self, lo, hi, shape):
        return jax.random.randint(self._next(), shape, lo, hi, dtype=jnp.int32)
    def uniform(self, shape, lo=0.0, hi=1.0):
        return jax.random.uniform(self._next(), shape, jnp.bfloat16, lo, hi)
    def permutation(self, n):
        return jax.random.permutation(self._next(), n)


kernel_name = 'gated_mix__mha_block_cached__gqa_block_cached__decode'

def setup_inputs():
    _rng = _Rng(jax.random.key(int.from_bytes(__import__("os").urandom(4), "little")))
    _w = (lambda a: (lambda t: t.astype(jnp.bfloat16) if jnp.issubdtype(t.dtype, jnp.floating) else t)(jnp.asarray(a)))
    def _A_setup():
        B, Sq, D = 4, 1, 512
        H, Sk, Dh = 32, 8192, 128
        return {
            "x": _w((lambda *s: _rng.normal(s) * 0.05)(B, Sq, D)),
            "k_cache": _w((lambda *s: _rng.normal(s) * 3.2)(B, H, Sk, Dh)),
            "v_cache": _w((lambda *s: _rng.normal(s) * 0.05)(B, H, Sk, Dh)),
            "wq": _w((lambda *s: _rng.normal(s) * 3.2)(D, H * Dh) * (D ** -0.5)),
            "wo": _w((lambda *s: _rng.normal(s) * 0.05)(H * Dh, D) * ((H * Dh) ** -0.5)),
        }
    _A_in = _A_setup()

    def _B_setup():
        B, Sq, D = 4, 1, 512
        Hq, Hkv, Sk, Dh = 32, 8, 8192, 128
        assert Hq % Hkv == 0, (Hq, Hkv)
        return {
            "x": _w((lambda *s: _rng.normal(s) * 0.05)(B, Sq, D)),
            "k_cache": _w((lambda *s: _rng.normal(s) * 3.2)(B, Hkv, Sk, Dh)),
            "v_cache": _w((lambda *s: _rng.normal(s) * 0.05)(B, Hkv, Sk, Dh)),
            "wq": _w((lambda *s: _rng.normal(s) * 3.2)(D, Hq * Dh) * (D ** -0.5)),
            "wo": _w((lambda *s: _rng.normal(s) * 0.05)(Hq * Dh, D) * ((Hq * Dh) ** -0.5)),
        }
    _B_in = _B_setup()

    return {
        "A_x": _A_in["x"],
        "A_k_cache": _A_in["k_cache"],
        "A_v_cache": _A_in["v_cache"],
        "A_wq": _A_in["wq"],
        "A_wo": _A_in["wo"],
        "B_x": _B_in["x"],
        "B_k_cache": _B_in["k_cache"],
        "B_v_cache": _B_in["v_cache"],
        "B_wq": _B_in["wq"],
        "B_wo": _B_in["wo"],
        "gate_w": _w((lambda *s: _rng.normal(s) * 0.05)(512) * 16.0),
    }

def reference(A_x, A_k_cache, A_v_cache, A_wq, A_wo, B_x, B_k_cache, B_v_cache, B_wq, B_wo, gate_w):
    def _A_ref(x, k_cache, v_cache, wq, wo):
        B, Sq, D = x.shape
        H, Dh = 32, 128
        q = (lambda x, *d: x.transpose(*d))((x @ wq).reshape(B, Sq, H, Dh), 0, 2, 1, 3)
        scores = jnp.einsum("bhqd,bhkd->bhqk", q, k_cache) * (Dh ** -0.5)
        p = _softmax(scores, axis=-1)
        o = jnp.einsum("bhqk,bhkd->bhqd", p, v_cache)
        return (lambda x, *d: x.transpose(*d))(o, 0, 2, 1, 3).reshape(B, Sq, H * Dh) @ wo

    def _B_ref(x, k_cache, v_cache, wq, wo):
        B, Sq, D = x.shape
        Hq, Dh = 32, 128
        Hkv = k_cache.shape[1]
        rep = Hq // Hkv
        q = (lambda x, *d: x.transpose(*d))((x @ wq).reshape(B, Sq, Hq, Dh), 0, 2, 1, 3)
        k = jnp.repeat(k_cache, rep, axis=1)
        v = jnp.repeat(v_cache, rep, axis=1)
        scores = jnp.einsum("bhqd,bhkd->bhqk", q, k) * (Dh ** -0.5)
        p = _softmax(scores, axis=-1)
        o = jnp.einsum("bhqk,bhkd->bhqd", p, v)
        return (lambda x, *d: x.transpose(*d))(o, 0, 2, 1, 3).reshape(B, Sq, Hq * Dh) @ wo

    x = A_x
    g = _sigmoid((x * gate_w).sum(-1, keepdims=True))
    a = _A_ref(x, A_k_cache, A_v_cache, A_wq, A_wo)
    b = _B_ref(x, B_k_cache, B_v_cache, B_wq, B_wo)
    return g * a + (1 - g) * b
```

```python
import functools
import jax, jax.numpy as jnp
from jax import lax
from jax.experimental import pallas as pl
from jax.experimental.pallas import tpu as pltpu

B, D, H, HKV, SK, DH = 4, 512, 32, 8, 8192, 128
REP = H // HKV
NS = 2
C = 128
J = SK // C
NVP = 8
VP = SK // NVP
NB_UNITS = B * HKV
NA_UNITS = B * H
N_UNITS = NA_UNITS + NB_UNITS
SCALE = DH ** -0.5
UNROLL = 8


def kernel(x_hbm, ak, av, awq, awo, bk, bv, bwq, bwo, gw_hbm, out_hbm,
           xbuf, gwbuf, wqbuf, wobuf, kbuf, vbuf, qa, qb, oa, ob, outbuf,
           sem_small, sem_w, sem_k, sem_v):
    f32 = jnp.float32
    bf16 = jnp.bfloat16

    def issue_kv(ksrc, vsrc, b, h, slot):
        per_piece = VP // C
        def body(pc, c):
            for e in range(per_piece):
                off = pl.multiple_of(pc * VP + e * C, C)
                pltpu.make_async_copy(ksrc.at[b, h, pl.ds(off, C)], kbuf.at[slot, pl.ds(off, C)],
                                      sem_k.at[slot]).start(priority=0)
                pltpu.make_async_copy(vsrc.at[b, h, pl.ds(off, C)], vbuf.at[slot, pl.ds(off, C)],
                                      sem_v.at[slot, pc]).start(priority=1)
            return c
        lax.fori_loop(0, NVP, body, 0)

    def wait_k(slot):
        pltpu.make_async_copy(kbuf.at[slot], kbuf.at[slot], sem_k.at[slot]).wait()

    def wait_v(slot, pc):
        pltpu.make_async_copy(vbuf.at[slot, pl.ds(pc * VP, VP)], vbuf.at[slot, pl.ds(pc * VP, VP)],
                              sem_v.at[slot, pc]).wait()

    def start_unit(u):
        slot = u % NS
        @pl.when(u < NB_UNITS)
        def _():
            issue_kv(bk, bv, u % B, u // B, slot)
        @pl.when(jnp.logical_and(u >= NB_UNITS, u < N_UNITS))
        def _():
            ua = u - NB_UNITS
            issue_kv(ak, av, ua % B, ua // B, slot)

    def issue_wq(src, idx, sem_i, lo, hi):
        def body(t, c):
            r = pl.multiple_of(t * 8, 8)
            pltpu.make_async_copy(src.at[pl.ds(r, 8), pl.ds(0, 2048)], wqbuf.at[idx, pl.ds(r, 8), pl.ds(0, 2048)],
                                  sem_w.at[sem_i]).start(priority=0)
            pltpu.make_async_copy(src.at[pl.ds(r, 8), pl.ds(2048, 2048)], wqbuf.at[idx, pl.ds(r, 8), pl.ds(2048, 2048)],
                                  sem_w.at[sem_i]).start(priority=1)
            return c
        lax.fori_loop(lo, hi, body, 0)

    def issue_wo(src, idx, sem_i, lo, hi):
        def body(t, c):
            r = pl.multiple_of(t * 64, 64)
            pltpu.make_async_copy(src.at[pl.ds(r, 32)], wobuf.at[idx, pl.ds(r, 32)], sem_w.at[sem_i]).start(priority=0)
            pltpu.make_async_copy(src.at[pl.ds(r + 32, 32)], wobuf.at[idx, pl.ds(r + 32, 32)], sem_w.at[sem_i]).start(priority=1)
            return c
        lax.fori_loop(lo, hi, body, 0)

    def wait_wq(idx, sem_i):
        pltpu.make_async_copy(wqbuf.at[idx], wqbuf.at[idx], sem_w.at[sem_i]).wait()

    def wait_wo(idx, sem_i):
        pltpu.make_async_copy(wobuf.at[idx], wobuf.at[idx], sem_w.at[sem_i]).wait()

    cx = pltpu.make_async_copy(x_hbm, xbuf, sem_small.at[0])
    cg = pltpu.make_async_copy(gw_hbm, gwbuf, sem_small.at[1])
    cx.start(); cg.start()
    issue_wq(bwq, 1, 0, 0, 64)
    start_unit(jnp.int32(0))

    cx.wait(); cg.wait()
    xf = xbuf[...].astype(f32)
    row16 = lax.broadcasted_iota(jnp.int32, (16, D), 0)
    row8 = lax.broadcasted_iota(jnp.int32, (8, D), 0)
    x16 = jnp.zeros((16, D), f32)
    x8 = jnp.zeros((8, D), f32)
    for b in range(B):
        x16 = jnp.where(row16 // 4 == b, jnp.broadcast_to(xf[b:b+1], (16, D)), x16)
        x8 = jnp.where(row8 == b, jnp.broadcast_to(xf[b:b+1], (8, D)), x8)
    gw = gwbuf[...].astype(f32).reshape(1, D)
    gate = jax.nn.sigmoid(jnp.sum(x8 * gw, axis=-1, keepdims=True))

    wait_wq(1, 0)
    qfull = jnp.dot(x16.astype(bf16), wqbuf[1], preferred_element_type=f32)
    r16 = lax.broadcasted_iota(jnp.int32, (16, DH), 0)
    for g in range(HKV):
        acc = jnp.zeros((16, DH), f32)
        for j in range(REP):
            hh = g * REP + j
            acc = jnp.where(r16 % 4 == j, qfull[:, hh*DH:(hh+1)*DH], acc)
        qb[g] = acc

    def attend(q, slot):
        wait_k(slot)
        s = lax.dot_general(q, kbuf[slot], (((1,), (1,)), ((), ())), preferred_element_type=f32)
        m = jnp.max(s, axis=-1, keepdims=True)
        p = jnp.exp((s - m) * SCALE)
        l = jnp.sum(p, axis=-1, keepdims=True)
        pb = p.astype(bf16)
        rl = 1.0 / l
        o = jnp.zeros((8, DH), f32)
        for pc in range(NVP):
            wait_v(slot, pc)
            o = o + jnp.dot(pb[:, pc*VP:(pc+1)*VP], vbuf[slot, pc*VP:(pc+1)*VP, :], preferred_element_type=f32)
        return o * rl

    def b_body(u, c):
        slot = u % NS
        g = u // B
        b = u % B
        start_unit(u + 1)
        @pl.when(u < 8)
        def _():
            issue_wq(awq, 0, 1, u * 8, u * 8 + 8)
        @pl.when(jnp.logical_and(u >= 8, u < 16))
        def _():
            issue_wo(bwo, 1, 2, (u - 8) * 8, (u - 8) * 8 + 8)
        @pl.when(jnp.logical_and(u >= 16, u < 24))
        def _():
            issue_wo(awo, 0, 3, (u - 16) * 8, (u - 16) * 8 + 8)
        half = pl.multiple_of((b // 2) * 8, 8)
        q = qb[g, pl.ds(half, 8), :].astype(bf16)
        o = attend(q, slot)
        r8 = lax.broadcasted_iota(jnp.int32, (8, DH), 0)
        old = ob[g, pl.ds(half, 8), :]
        ob[g, pl.ds(half, 8), :] = jnp.where(r8 // 4 == b % 2, o, old)
        return c
    ob[...] = jnp.zeros(ob.shape, f32)
    oa[...] = jnp.zeros(oa.shape, f32)
    lax.fori_loop(0, NB_UNITS - 8, b_body, 0)

    wait_wq(0, 1)
    qfa = jnp.dot(x8.astype(bf16), wqbuf[0], preferred_element_type=f32)
    for h in range(H):
        qa[h] = qfa[:, h*DH:(h+1)*DH]
    lax.fori_loop(NB_UNITS - 8, NB_UNITS, b_body, 0)

    def a_body(ua, acc):
        u = ua + NB_UNITS
        slot = u % NS
        h = ua // B
        b = ua % B
        start_unit(u + 1)
        q = qa[h].astype(bf16)
        o = attend(q, slot)
        r8 = lax.broadcasted_iota(jnp.int32, (8, DH), 0)
        oa[h] = jnp.where(r8 == b, o, oa[h])
        return acc
    lax.fori_loop(0, 4, a_body, 0)

    wait_wo(1, 2)
    r16o = lax.broadcasted_iota(jnp.int32, (16, DH), 0)
    accb = jnp.zeros((16, D), f32)
    for g in range(HKV):
        og = ob[g]
        for j in range(REP):
            hh = g * REP + j
            lhs = jnp.where(r16o % 4 == j, og, 0.0).astype(bf16)
            accb = accb + jnp.dot(lhs, wobuf[1, hh*DH:(hh+1)*DH, :], preferred_element_type=f32)
    r16d = lax.broadcasted_iota(jnp.int32, (16, D), 0)
    outb = jnp.zeros((8, D), f32)
    for b in range(B):
        ob_b = jnp.sum(jnp.where(r16d // 4 == b, accb, 0.0), axis=0, keepdims=True)
        outb = jnp.where(row8 == b, jnp.broadcast_to(ob_b, (8, D)), outb)
    partial = (1.0 - gate) * outb

    lax.fori_loop(4, NA_UNITS - 4, a_body, 0)
    wait_wo(0, 3)
    acca = jnp.zeros((8, D), f32)
    for h in range(H - 1):
        acca = acca + jnp.dot(oa[h].astype(bf16), wobuf[0, h*DH:(h+1)*DH, :], preferred_element_type=f32)
    lax.fori_loop(NA_UNITS - 4, NA_UNITS, a_body, 0)
    h = H - 1
    acca = acca + jnp.dot(oa[h].astype(bf16), wobuf[0, h*DH:(h+1)*DH, :], preferred_element_type=f32)
    res = gate * acca + partial
    outbuf[...] = res[0:B].astype(bf16)
    co = pltpu.make_async_copy(outbuf, out_hbm, sem_small.at[2])
    co.start()
    co.wait()


@jax.jit
def pallas_gated_mix__mha_block_cached__gqa_block_cached__decode_kernel(A_x, A_k_cache, A_v_cache, A_wq, A_wo, B_x, B_k_cache, B_v_cache, B_wq, B_wo, gate_w):
    bf16 = jnp.bfloat16
    f32 = jnp.float32
    any_spec = pl.BlockSpec(memory_space=pl.ANY)
    out = pl.pallas_call(
        kernel,
        in_specs=[any_spec] * 10,
        out_specs=any_spec,
        out_shape=jax.ShapeDtypeStruct((B, D), bf16),
        scratch_shapes=[
            pltpu.VMEM((B, D), bf16),
            pltpu.VMEM((D,), bf16),
            pltpu.VMEM((2, D, H * DH), bf16),
            pltpu.VMEM((2, H * DH, D), bf16),
            pltpu.VMEM((NS, SK, DH), bf16),
            pltpu.VMEM((NS, SK, DH), bf16),
            pltpu.VMEM((H, 8, DH), f32),
            pltpu.VMEM((HKV, 16, DH), f32),
            pltpu.VMEM((H, 8, DH), f32),
            pltpu.VMEM((HKV, 16, DH), f32),
            pltpu.VMEM((B, D), bf16),
            pltpu.SemaphoreType.DMA((3,)),
            pltpu.SemaphoreType.DMA((4,)),
            pltpu.SemaphoreType.DMA((NS,)),
            pltpu.SemaphoreType.DMA((NS, NVP)),
        ],
        compiler_params=pltpu.CompilerParams(vmem_limit_bytes=100 * 1024 * 1024, disable_bounds_checks=True),
    )(A_x.reshape(B, D), A_k_cache, A_v_cache, A_wq, A_wo, B_k_cache, B_v_cache, B_wq, B_wo, gate_w)
    return out.reshape(B, 1, D)
```

```python
import functools, os
import jax, jax.numpy as jnp
from jax import lax
from jax.experimental import pallas as pl
from jax.experimental.pallas import tpu as pltpu

B, D, H, HKV, SK, DH = 4, 512, 32, 8, 8192, 128
G = 8
R = int(os.environ.get("R", "512"))
C = int(os.environ.get("C", "64"))
NS = 2
NBLK = SK // R
NCH = R // C
T_B = B * NBLK
T_A = B * (H // G) * NBLK
T = T_A + T_B
SCALE = DH ** -0.5
NOCOMP = int(os.environ.get("NOCOMP", "0"))
DBC = int(os.environ.get("DBC", "0"))


def kernel(x_hbm, ak, av, awq, awo, bk, bv, bwq, bwo, gw_hbm, out_hbm,
           xbuf, gwbuf, wqbuf, wobuf, kbuf, vbuf, qbuf, m_ref, l_ref, acc_ref, oacc, outbuf,
           sem_small, sem_w, sem_k, sem_v):
    f32 = jnp.float32
    bf16 = jnp.bfloat16

    def issue_half(ksrc, vsrc, b, h0, j, slot, half, v_head_major):
        def body(cc, c):
            for i in range(G):
                koff = pl.multiple_of(cc * C, C)
                pltpu.make_async_copy(
                    ksrc.at[b, h0 + i, pl.ds(j * R + koff, C)],
                    kbuf.at[slot, i, pl.ds(koff, C)], sem_k.at[slot]).start(priority=0)
                if v_head_major:
                    k = cc * G + i
                    vh = k // NCH
                    voff = pl.multiple_of((k % NCH) * C, C)
                else:
                    vh = i
                    voff = koff
                pltpu.make_async_copy(
                    vsrc.at[b, h0 + vh, pl.ds(j * R + voff, C)],
                    vbuf.at[slot, vh, pl.ds(voff, C)], sem_v.at[slot, vh]).start(priority=1)
            return c
        lax.fori_loop(half * (NCH // 2), (half + 1) * (NCH // 2), body, 0)

    def issue_step(t, half):
        slot = t % NS
        j = t % NBLK
        @pl.when(t < T_B)
        def _():
            issue_half(bk, bv, t // NBLK, 0, j, slot, half, False)
        @pl.when(jnp.logical_and(t >= T_B, t < T - 1))
        def _():
            g = (t - T_B) // NBLK
            issue_half(ak, av, g // (H // G), (g % (H // G)) * G, j, slot, half, False)
        @pl.when(t == T - 1)
        def _():
            issue_half(ak, av, B - 1, H - G, NBLK - 1, slot, half, True)

    def wait_k(slot):
        pltpu.make_async_copy(kbuf.at[slot], kbuf.at[slot], sem_k.at[slot]).wait()

    def wait_v(slot, i):
        pltpu.make_async_copy(vbuf.at[slot, i], vbuf.at[slot, i], sem_v.at[slot, i]).wait()

    def issue_weights():
        def body(k, c):
            for s in range(8):
                a, reg = s // 4, s % 4
                wq_src = (bwq, awq)[a]
                wo_src = (bwo, awo)[a]
                r = pl.multiple_of(reg * 128 + (k // 4) * 8, 8)
                cc = pl.multiple_of((k % 4) * 1024, 1024)
                pltpu.make_async_copy(wq_src.at[pl.ds(r, 8), pl.ds(cc, 1024)],
                                      wqbuf.at[a, pl.ds(r, 8), pl.ds(cc, 1024)], sem_w.at[a]).start(priority=0)
                ro = pl.multiple_of(reg * 1024 + k * 16, 16)
                pltpu.make_async_copy(wo_src.at[pl.ds(ro, 16)], wobuf.at[a, pl.ds(ro, 16)],
                                      sem_w.at[2 + a]).start(priority=1)
            return c
        lax.fori_loop(0, 64, body, 0)

    def wait_wq(a):
        pltpu.make_async_copy(wqbuf.at[a], wqbuf.at[a], sem_w.at[a]).wait()

    def wait_wo(a):
        pltpu.make_async_copy(wobuf.at[a], wobuf.at[a], sem_w.at[2 + a]).wait()

    cx = pltpu.make_async_copy(x_hbm, xbuf, sem_small.at[0])
    cg = pltpu.make_async_copy(gw_hbm, gwbuf, sem_small.at[1])
    cx.start(); cg.start()
    issue_weights()
    issue_step(jnp.int32(0), 0)

    cx.wait(); cg.wait()
    xf = xbuf[...].astype(f32)
    row8d = lax.broadcasted_iota(jnp.int32, (8, D), 0)
    x8 = jnp.zeros((8, D), f32)
    for b in range(B):
        x8 = jnp.where(row8d == b, jnp.broadcast_to(xf[b:b+1], (8, D)), x8)
    gw = gwbuf[...].astype(f32).reshape(1, D)
    gate = jax.nn.sigmoid(jnp.sum(x8 * gw, axis=-1, keepdims=True))
    x32 = jnp.concatenate([jnp.broadcast_to(xf[b:b+1], (8, D)) for b in range(B)], axis=0).astype(bf16)
    row8 = lax.broadcasted_iota(jnp.int32, (8, DH), 0)

    def compute_q(a):
        for hg in range(H // G):
            res = jnp.dot(x32, wqbuf[a, :, hg * G * DH:(hg + 1) * G * DH], preferred_element_type=f32)
            for b in range(B):
                q = res[8 * b:8 * b + 8, 0:DH]
                for r in range(1, G):
                    q = jnp.where(row8 == r, res[8 * b:8 * b + 8, r * DH:(r + 1) * DH], q)
                qbuf[a, b * (H // G) + hg] = q

    wait_wq(0)
    compute_q(0)
    issue_step(jnp.int32(0), 1)
    wait_wq(1)
    compute_q(1)
    oacc[...] = jnp.zeros(oacc.shape, f32)
    wait_wo(0)
    wait_wo(1)

    def scores(phase, qs, slot):
        NP = 4 if phase == 0 else 1
        S = [None] * NP
        for i in range(G):
            p = i // 2 if phase == 0 else 0
            s = lax.dot_general(qs[p], kbuf[slot, i], (((1,), (1,)), ((), ())), preferred_element_type=f32)
            if S[p] is None:
                S[p] = s
            else:
                rr = lax.broadcasted_iota(jnp.int32, (8, R), 0)
                valid = (rr // 4 == i % 2) if phase == 0 else (rr == i)
                S[p] = jnp.where(valid, s, S[p])
        return S

    def softmax_update(phase, S):
        NP = len(S)
        P, alphas = [], []
        for p in range(NP):
            m_old = m_ref[p]
            m_new = jnp.maximum(m_old, jnp.max(S[p], axis=1, keepdims=True))
            alpha = jnp.exp((m_old - m_new) * SCALE)
            pr = jnp.exp((S[p] - m_new[:, 0:1]) * SCALE)
            lsum = pr[:, 0:128]
            for c in range(1, R // 128):
                lsum = lsum + pr[:, c * 128:(c + 1) * 128]
            l_ref[p] = alpha * l_ref[p] + lsum
            m_ref[p] = m_new
            P.append(pr.astype(bf16))
            alphas.append(alpha)
        return P, alphas

    def project(phase, p, o, head0):
        ob = o.astype(bf16)
        out = None
        for r in range(G):
            hrow = pl.multiple_of((head0 + 8 * p + r) * DH, DH)
            y = jnp.dot(ob, wobuf[phase, pl.ds(hrow, DH), :], preferred_element_type=f32)
            out = y if out is None else jnp.where(row8d == r, y, out)
        return out

    def step(phase, t):
        slot = t % NS
        j = t % NBLK
        NP = 4 if phase == 0 else 1
        if phase == 0:
            b = t // NBLK
            hg0 = 0
        else:
            g = (t - T_B) // NBLK
            b = g // (H // G)
            hg0 = g % (H // G)
        issue_step(t + 1, 0)

        @pl.when(j == 0)
        def _():
            m_ref[...] = jnp.full(m_ref.shape, -jnp.inf, f32)
            l_ref[...] = jnp.zeros(l_ref.shape, f32)
            acc_ref[...] = jnp.zeros(acc_ref.shape, f32)

        qs = [qbuf[phase, b * (H // G) + hg0 + p].astype(bf16) for p in range(NP)]
        wait_k(slot)
        if not NOCOMP:
            S = scores(phase, qs, slot)
            P, alphas = softmax_update(phase, S)
        issue_step(t + 1, 1)
        for i in range(G):
            wait_v(slot, i)
        if NOCOMP:
            return
        PV = [None] * NP
        for i in range(G):
            p = i // 2 if phase == 0 else 0
            o = jnp.dot(P[p], vbuf[slot, i], preferred_element_type=f32)
            if PV[p] is None:
                PV[p] = o
            else:
                valid = (row8 // 4 == i % 2) if phase == 0 else (row8 == i)
                PV[p] = jnp.where(valid, o, PV[p])
        for p in range(NP):
            acc_ref[p] = alphas[p] * acc_ref[p] + PV[p]

        @pl.when(j == NBLK - 1)
        def _():
            tot = None
            for p in range(NP):
                l = jnp.sum(l_ref[p], axis=1, keepdims=True)
                y = project(phase, p, acc_ref[p] / l, hg0 * G)
                tot = y if tot is None else tot + y
            row = jnp.sum(tot, axis=0, keepdims=True)
            oacc[phase] = oacc[phase] + jnp.where(row8d == b, jnp.broadcast_to(row, (8, D)), 0.0)

    def loop(phase, lo, hi):
        def body(t, c):
            step(phase, t)
            return c
        lax.fori_loop(lo, hi, body, 0)

    loop(0, 0, T_B)
    loop(1, T_B, T - 1)

    t = T - 1
    slot = t % NS
    b = B - 1
    hg0 = H // G - 1
    q = qbuf[1, b * (H // G) + hg0].astype(bf16)
    wait_k(slot)
    S = scores(1, [q], slot)
    P, alphas = softmax_update(1, S)
    l = jnp.sum(l_ref[0], axis=1, keepdims=True)
    rl = 1.0 / l
    prev = alphas[0] * acc_ref[0]
    tot = None
    for grp in ((0, 1, 2, 3, 4, 5), (6, 7)):
        for i in grp:
            wait_v(slot, i)
        for i in grp:
            o = (prev + jnp.dot(P[0], vbuf[slot, i], preferred_element_type=f32)) * rl
            hrow = (hg0 * G + i) * DH
            y = jnp.dot(o.astype(bf16), wobuf[1, hrow:hrow + DH, :], preferred_element_type=f32)
            tot = y if tot is None else jnp.where(row8d == i, y, tot)
    row = jnp.sum(tot, axis=0, keepdims=True)
    outa = oacc[1] + jnp.where(row8d == b, jnp.broadcast_to(row, (8, D)), 0.0)
    res = gate * outa + (1.0 - gate) * oacc[0]
    outbuf[...] = res[0:B].astype(bf16)
    co = pltpu.make_async_copy(outbuf, out_hbm, sem_small.at[2])
    co.start()
    co.wait()


@jax.jit
def pallas_gated_mix__mha_block_cached__gqa_block_cached__decode_kernel(A_x, A_k_cache, A_v_cache, A_wq, A_wo, B_x, B_k_cache, B_v_cache, B_wq, B_wo, gate_w):
    bf16 = jnp.bfloat16
    f32 = jnp.float32
    any_spec = pl.BlockSpec(memory_space=pl.ANY)
    out = pl.pallas_call(
        kernel,
        in_specs=[any_spec] * 10,
        out_specs=any_spec,
        out_shape=jax.ShapeDtypeStruct((B, D), bf16),
        scratch_shapes=[
            pltpu.VMEM((B, D), bf16),
            pltpu.VMEM((D,), bf16),
            pltpu.VMEM((2, D, H * DH), bf16),
            pltpu.VMEM((2, H * DH, D), bf16),
            pltpu.VMEM((NS, G, R, DH), bf16),
            pltpu.VMEM((NS, G, R, DH), bf16),
            pltpu.VMEM((2, B * H // G, 8, DH), f32),
            pltpu.VMEM((4, 8, 128), f32),
            pltpu.VMEM((4, 8, 128), f32),
            pltpu.VMEM((4, 8, DH), f32),
            pltpu.VMEM((2, 8, D), f32),
            pltpu.VMEM((B, D), bf16),
            pltpu.SemaphoreType.DMA((3,)),
            pltpu.SemaphoreType.DMA((4,)),
            pltpu.SemaphoreType.DMA((NS,)),
            pltpu.SemaphoreType.DMA((NS, G)),
        ],
        compiler_params=pltpu.CompilerParams(vmem_limit_bytes=100 * 1024 * 1024, disable_bounds_checks=bool(DBC)),
    )(A_x.reshape(B, D), A_k_cache, A_v_cache, A_wq, A_wo, B_k_cache, B_v_cache, B_wq, B_wo, gate_w)
    return out.reshape(B, 1, D)
```

```python
import functools, os
import contextlib
import jax, jax.numpy as jnp
from jax import lax
from jax.experimental import pallas as pl
from jax.experimental.pallas import tpu as pltpu

B, D, H, HKV, SK, DH = 4, 512, 32, 8, 8192, 128
G = 8
R = 512
C = 64
NS = 3
NBLK = SK // R
NCH = R // C
HG = H // G
T_B = B * NBLK
T_A = B * HG * NBLK
T = T_A + T_B
SCALE = DH ** -0.5
DBC = int(os.environ.get("DBC", "1"))
VLP = int(os.environ.get("VLP", "1"))
SCOPES = int(os.environ.get("SCOPES", "0"))
POS = [int(v) for v in os.environ.get("POS", "0,2,4,6,8,10,12,14").split(",")]


def scope(name):
    return jax.named_scope(name) if SCOPES else contextlib.nullcontext()


def kernel(x_hbm, ak, av, awq, awo, bk, bv, bwq, bwo, gw_hbm, out_hbm,
           xbuf, gwbuf, wqbuf, wobuf, kvbuf, qbuf, m_ref, l_ref, a_ref, p_ref, acc_ref, oacc, outbuf,
           sem_small, sem_w, sem_k, sem_v, sem_vl):
    f32 = jnp.float32
    bf16 = jnp.bfloat16

    def coords(kind, t):
        if kind == 'B':
            return t // NBLK, 0, t % NBLK
        g = (t - T_B) // NBLK
        return g // HG, (g % HG) * G, t % NBLK

    def start_k(kind, t, i, cc, prio):
        b, h0, j = coords(kind, t)
        src = bk if kind == 'B' else ak
        pltpu.make_async_copy(src.at[b, h0 + i, pl.ds(j * R + cc * C, C)],
                              kvbuf.at[0, t % NS, i, pl.ds(cc * C, C)], sem_k.at[t % NS]).start(priority=prio)

    def start_v(kind, t, i, cc, prio, sem=None):
        b, h0, j = coords(kind, t)
        src = bv if kind == 'B' else av
        pltpu.make_async_copy(src.at[b, h0 + i, pl.ds(j * R + cc * C, C)],
                              kvbuf.at[1, t % NS, i, pl.ds(cc * C, C)],
                              sem_v.at[t % NS] if sem is None else sem).start(priority=prio)

    def plan_pair(kk, tk, kv, tv):
        def grp(cc):
            for i in range(G):
                start_k(kk, tk, i, cc, 0)
                start_v(kv, tv, i, cc, 1)
        return [functools.partial(grp, cc) for cc in range(NCH)]

    def plan_only(start, kind, t):
        def grp(g):
            for cc in (2 * g, 2 * g + 1):
                for i in range(G):
                    start(kind, t, i, cc, i % 2)
        return [functools.partial(grp, g) for g in range(NCH // 2)]

    def plan_vlast(t):
        def grp(g):
            for cc in range(NCH):
                for i in (2 * g, 2 * g + 1):
                    start_v('A', t, i, cc, VLP if VLP >= 0 else i % 2, sem_vl.at[g])
        return [functools.partial(grp, g) for g in range(G // 2)]

    def wait_k(t):
        s = t % NS
        pltpu.make_async_copy(kvbuf.at[0, s], kvbuf.at[0, s], sem_k.at[s]).wait()

    def wait_v(t):
        s = t % NS
        pltpu.make_async_copy(kvbuf.at[1, s], kvbuf.at[1, s], sem_v.at[s]).wait()

    def wait_vl(t, g):
        buf = kvbuf.at[1, t % NS, pl.ds(2 * g, 2)]
        pltpu.make_async_copy(buf, buf, sem_vl.at[g]).wait()

    def issue_wq(lo, hi):
        def body(k, c):
            for reg in range(4):
                r = pl.multiple_of(reg * 128 + (k // 4) * 8, 8)
                cc = pl.multiple_of((k % 4) * 1024, 1024)
                for a, src in enumerate((bwq, awq)):
                    pltpu.make_async_copy(src.at[pl.ds(r, 8), pl.ds(cc, 1024)],
                                          wqbuf.at[a, pl.ds(r, 8), pl.ds(cc, 1024)], sem_w.at[a]).start(priority=a)
            return c
        lax.fori_loop(lo, hi, body, 0)

    def issue_wo(lo, hi):
        def body(k, c):
            for reg in range(4):
                r = pl.multiple_of(reg * 1024 + k * 16, 16)
                for a, src in enumerate((bwo, awo)):
                    pltpu.make_async_copy(src.at[pl.ds(r, 16)], wobuf.at[a, pl.ds(r, 16)],
                                          sem_w.at[2 + a]).start(priority=a)
            return c
        lax.fori_loop(lo, hi, body, 0)

    def wait_wq(a):
        pltpu.make_async_copy(wqbuf.at[a], wqbuf.at[a], sem_w.at[a]).wait()

    def wait_wo(a):
        pltpu.make_async_copy(wobuf.at[a], wobuf.at[a], sem_w.at[2 + a]).wait()

    row8 = lax.broadcasted_iota(jnp.int32, (8, DH), 0)
    row8d = lax.broadcasted_iota(jnp.int32, (8, D), 0)

    def q_index(kind, t):
        b, h0, _ = coords(kind, t)
        return b * HG + h0 // G

    def load_q(kind, t):
        ph = 0 if kind == 'B' else 1
        base = q_index(kind, t)
        return [qbuf[ph, base + p].astype(bf16) for p in range(4 if kind == 'B' else 1)]

    def qk_head(kind, qs, t, i, S):
        p = i // 2 if kind == 'B' else 0
        s = lax.dot_general(qs[p], kvbuf[0, t % NS, i], (((1,), (1,)), ((), ())), preferred_element_type=f32)
        if S[p] is None:
            S[p] = s
        else:
            rr = lax.broadcasted_iota(jnp.int32, (8, R), 0)
            valid = (rr // 4 == i % 2) if kind == 'B' else (rr == i)
            S[p] = jnp.where(valid, s, S[p])

    def softmax_update(S, first):
        for p in range(len(S)):
            m_old = jnp.where(first, -jnp.inf, m_ref[p])
            l_old = jnp.where(first, 0.0, l_ref[p])
            m_new = jnp.maximum(m_old, jnp.max(S[p], axis=1, keepdims=True))
            alpha = jnp.exp((m_old - m_new) * SCALE)
            pr = jnp.exp((S[p] - m_new[:, 0:1]) * SCALE)
            lsum = pr[:, 0:128]
            for c in range(1, R // 128):
                lsum = lsum + pr[:, c * 128:(c + 1) * 128]
            l_ref[p] = alpha * l_old + lsum
            m_ref[p] = m_new
            a_ref[p] = alpha
            p_ref[p] = pr.astype(bf16)

    def pv_head(kind, P, t, i, PV):
        p = i // 2 if kind == 'B' else 0
        o = jnp.dot(P[p], kvbuf[1, t % NS, i], preferred_element_type=f32)
        if PV[p] is None:
            PV[p] = o
        else:
            valid = (row8 // 4 == i % 2) if kind == 'B' else (row8 == i)
            PV[p] = jnp.where(valid, o, PV[p])

    def project(ph, o, head0):
        ob = o.astype(bf16)
        out = None
        for r in range(G):
            hrow = pl.multiple_of((head0 + r) * DH, DH)
            y = jnp.dot(ob, wobuf[ph, pl.ds(hrow, DH), :], preferred_element_type=f32)
            out = y if out is None else jnp.where(row8d == r, y, out)
        return out

    def step(pv, qk, plan, t, pos=None, late_v=False):
        pos = POS if pos is None else pos

        def issue_at(p):
            for g, thunk in enumerate(plan):
                if pos[g] == p:
                    thunk()

        NP = 4 if pv == 'B' else 1
        P = [p_ref[p] for p in range(NP)]
        alphas = [a_ref[p] for p in range(NP)]
        l_cur = [l_ref[p] for p in range(NP)]
        if qk is not None:
            qs = load_q(qk, t + 1)
            wait_k(t + 1)
        if not late_v:
            wait_v(t)
        if qk is not None:
            S = [None] * (4 if qk == 'B' else 1)
            for i in range(G):
                issue_at(i)
                qk_head(qk, qs, t + 1, i, S)
        if late_v:
            with scope("lv_sm"):
                softmax_update(S, (t + 1) % NBLK == 0)
            with scope("lv_wait"):
                wait_v(t)
        PV = [None] * NP
        for i in range(G):
            issue_at(8 + i)
            pv_head(pv, P, t, i, PV)
        if qk is not None and not late_v:
            softmax_update(S, (t + 1) % NBLK == 0)
        first = t % NBLK == 0
        for p in range(NP):
            acc_ref[p] = jnp.where(first, PV[p], alphas[p] * acc_ref[p] + PV[p])
        issue_at(16)

        @pl.when(t % NBLK == NBLK - 1)
        def _():
            b, h0, _ = coords(pv, t)
            tot = None
            for p in range(NP):
                l = jnp.sum(l_cur[p], axis=1, keepdims=True)
                y = project(0 if pv == 'B' else 1, acc_ref[p] / l, h0 + 8 * p)
                tot = y if tot is None else tot + y
            row = jnp.sum(tot, axis=0, keepdims=True)
            ph = 0 if pv == 'B' else 1
            oacc[ph] = oacc[ph] + jnp.where(row8d == b, jnp.broadcast_to(row, (8, D)), 0.0)

    with scope("p_wq"):
        cx = pltpu.make_async_copy(x_hbm, xbuf, sem_small.at[0])
        cg = pltpu.make_async_copy(gw_hbm, gwbuf, sem_small.at[1])
        cx.start(); cg.start()
        issue_wq(0, 64)
        issue_wo(0, 16)

    with scope("p_x"):
        cx.wait(); cg.wait()
        xf = xbuf[...].astype(f32)
        x8 = jnp.zeros((8, D), f32)
        for b in range(B):
            x8 = jnp.where(row8d == b, jnp.broadcast_to(xf[b:b+1], (8, D)), x8)
        gw = gwbuf[...].astype(f32).reshape(1, D)
        gate = jax.nn.sigmoid(jnp.sum(x8 * gw, axis=-1, keepdims=True))
        x32 = jnp.concatenate([jnp.broadcast_to(xf[b:b+1], (8, D)) for b in range(B)], axis=0).astype(bf16)
        for ref in (m_ref, l_ref, a_ref, acc_ref, oacc):
            ref[...] = jnp.zeros(ref.shape, f32)

    def compute_q(a, hg):
        res = jnp.dot(x32, wqbuf[a, :, hg * G * DH:(hg + 1) * G * DH], preferred_element_type=f32)
        for b in range(B):
            q = res[8 * b:8 * b + 8, 0:DH]
            for r in range(1, G):
                q = jnp.where(row8 == r, res[8 * b:8 * b + 8, r * DH:(r + 1) * DH], q)
            qbuf[a, b * HG + hg] = q

    with scope("p_q"):
        wait_wq(0)
        wait_wq(1)
        for n in range(8):
            compute_q(n // HG, n % HG)
            issue_wo(16 + 6 * n, 16 + 6 * (n + 1))
    with scope("p_kv"):
        for thunk in plan_only(start_k, 'B', 0) + plan_pair('B', 1, 'B', 0) + plan_pair('B', 2, 'B', 1):
            thunk()
    with scope("p_qk0"):
        qs = load_q('B', 0)
        wait_k(0)
        S = [None] * 4
        for i in range(G):
            qk_head('B', qs, 0, i, S)
        softmax_update(S, True)
        wait_wo(0)
        wait_wo(1)

    def loop(pv, qk, kk, kv, lo, hi):
        def body(t, c):
            with scope("step"):
                step(pv, qk, plan_pair(kk, t + 3, kv, t + 2), t)
            return c
        lax.fori_loop(lo, hi, body, 0)

    def single(name, pv, qk, plan, t, pos=None, late_v=False):
        with scope(name):
            step(pv, qk, plan, t, pos, late_v)

    loop('B', 'B', 'B', 'B', 0, T_B - 3)
    t = T_B - 3
    single("s61", 'B', 'B', plan_pair('A', t + 3, 'B', t + 2), t)
    single("s62", 'B', 'B', plan_pair('A', t + 4, 'A', t + 3), t + 1)
    single("s63", 'B', 'A', plan_pair('A', t + 5, 'A', t + 4), t + 2)
    loop('A', 'A', 'A', 'A', T_B, T - 4)
    single("sT4", 'A', 'A', plan_only(start_k, 'A', T - 1) + plan_only(start_v, 'A', T - 2), T - 4)
    single("sT3", 'A', 'A', plan_vlast(T - 1), T - 3, pos=[8, 10, 12, 14])
    single("sT2", 'A', 'A', [], T - 2, late_v=True)

    t = T - 1
    b, h0, _ = coords('A', t)
    with scope("t_pre"):
        P = p_ref[0]
        rl = 1.0 / jnp.sum(l_ref[0], axis=1, keepdims=True)
        prev = a_ref[0] * acc_ref[0]
    tot = None
    for g in range(G // 2):
        with scope(f"t_pv{g}"):
            with scope(f"t_w{g}"):
                wait_vl(t, g)
            for i in (2 * g, 2 * g + 1):
                o = (prev + jnp.dot(P, kvbuf[1, t % NS, i], preferred_element_type=f32)) * rl
                hrow = (h0 + i) * DH
                y = jnp.dot(o.astype(bf16), wobuf[1, hrow:hrow + DH, :], preferred_element_type=f32)
                tot = y if tot is None else jnp.where(row8d == i, y, tot)
    with scope("t_fin"):
        row = jnp.sum(tot, axis=0, keepdims=True)
        outa = oacc[1] + jnp.where(row8d == b, jnp.broadcast_to(row, (8, D)), 0.0)
        res = gate * outa + (1.0 - gate) * oacc[0]
        outbuf[...] = res[0:B].astype(bf16)
    with scope("outdma"):
        co = pltpu.make_async_copy(outbuf, out_hbm, sem_small.at[2])
        co.start()
        co.wait()


@jax.jit
def pallas_gated_mix__mha_block_cached__gqa_block_cached__decode_kernel(A_x, A_k_cache, A_v_cache, A_wq, A_wo, B_x, B_k_cache, B_v_cache, B_wq, B_wo, gate_w):
    bf16 = jnp.bfloat16
    f32 = jnp.float32
    any_spec = pl.BlockSpec(memory_space=pl.ANY)
    out = pl.pallas_call(
        kernel,
        in_specs=[any_spec] * 10,
        out_specs=any_spec,
        out_shape=jax.ShapeDtypeStruct((B, D), bf16),
        scratch_shapes=[
            pltpu.VMEM((B, D), bf16),
            pltpu.VMEM((D,), bf16),
            pltpu.VMEM((2, D, H * DH), bf16),
            pltpu.VMEM((2, H * DH, D), bf16),
            pltpu.VMEM((2, NS, G, R, DH), bf16),
            pltpu.VMEM((2, B * HG, 8, DH), f32),
            pltpu.VMEM((4, 8, 128), f32),
            pltpu.VMEM((4, 8, 128), f32),
            pltpu.VMEM((4, 8, 128), f32),
            pltpu.VMEM((4, 8, R), bf16),
            pltpu.VMEM((4, 8, DH), f32),
            pltpu.VMEM((2, 8, D), f32),
            pltpu.VMEM((B, D), bf16),
            pltpu.SemaphoreType.DMA((3,)),
            pltpu.SemaphoreType.DMA((4,)),
            pltpu.SemaphoreType.DMA((NS,)),
            pltpu.SemaphoreType.DMA((NS,)),
            pltpu.SemaphoreType.DMA((G // 2,)),
        ],
        compiler_params=pltpu.CompilerParams(vmem_limit_bytes=100 * 1024 * 1024, disable_bounds_checks=bool(DBC)),
    )(A_x.reshape(B, D), A_k_cache, A_v_cache, A_wq, A_wo, B_k_cache, B_v_cache, B_wq, B_wo, gate_w)
    return out.reshape(B, 1, D)
```

```python
import functools, os
import contextlib
import jax, jax.numpy as jnp
from jax import lax
from jax.experimental import pallas as pl
from jax.experimental.pallas import tpu as pltpu

B, D, H, HKV, SK, DH = 4, 512, 32, 8, 8192, 128
G = 8
R = 512
C = 64
NS = 3
NBLK = SK // R
SR = int(os.environ.get('SR', '16'))
NQ = R // SR
NGRP = 8
HG = H // G
T_B = B * NBLK
T_A = B * HG * NBLK
T = T_A + T_B
SCALE = DH ** -0.5
DBC = int(os.environ.get("DBC", "1"))
VLP = int(os.environ.get("VLP", "1"))
SCOPES = int(os.environ.get("SCOPES", "0"))
POS = [int(v) for v in os.environ.get("POS", "0,2,4,6,8,10,12,14").split(",")]


def scope(name):
    return jax.named_scope(name) if SCOPES else contextlib.nullcontext()


def kernel(x_hbm, ak, av, awq, awo, bk, bv, bwq, bwo, gw_hbm, out_hbm,
           xbuf, gwbuf, wqbuf, wobuf, kvbuf, qbuf, m_ref, l_ref, a_ref, p_ref, acc_ref, oacc, outbuf,
           sem_small, sem_w, sem_k, sem_v, sem_vl):
    f32 = jnp.float32
    bf16 = jnp.bfloat16

    def coords(kind, t):
        if kind == 'B':
            return t // NBLK, 0, t % NBLK
        g = (t - T_B) // NBLK
        return g // HG, (g % HG) * G, t % NBLK

    def start_kv(which, kind, t, q, prio):
        b, h0, j = coords(kind, t)
        src = ((bk, bv) if kind == 'B' else (ak, av))[which]
        sem = (sem_k, sem_v)[which]
        pltpu.make_async_copy(src.at[b, pl.ds(h0, G), pl.ds(j * R + q * SR, SR)],
                              kvbuf.at[which, t % NS, :, pl.ds(q * SR, SR)], sem.at[t % NS]).start(priority=prio)

    def plan_pair(kk, tk, kv, tv):
        def grp(g):
            for q in range(g * NQ // NGRP, (g + 1) * NQ // NGRP):
                start_kv(0, kk, tk, q, 0)
                start_kv(1, kv, tv, q, 1)
        return [functools.partial(grp, g) for g in range(NGRP)]

    def plan_only(which, kind, t):
        def grp(g):
            for q in range(g * NQ // 4, (g + 1) * NQ // 4):
                start_kv(which, kind, t, q, q % 2)
        return [functools.partial(grp, g) for g in range(4)]

    def plan_vlast(t):
        b, h0, j = coords('A', t)
        def grp(g):
            for cc in range(R // C):
                for i in (2 * g, 2 * g + 1):
                    pltpu.make_async_copy(av.at[b, h0 + i, pl.ds(j * R + cc * C, C)],
                                          kvbuf.at[1, t % NS, i, pl.ds(cc * C, C)], sem_vl.at[g]).start(priority=1)
        return [functools.partial(grp, g) for g in range(G // 2)]

    def wait_k(t):
        s = t % NS
        pltpu.make_async_copy(kvbuf.at[0, s], kvbuf.at[0, s], sem_k.at[s]).wait()

    def wait_v(t):
        s = t % NS
        pltpu.make_async_copy(kvbuf.at[1, s], kvbuf.at[1, s], sem_v.at[s]).wait()

    def wait_vl(t, g):
        buf = kvbuf.at[1, t % NS, pl.ds(2 * g, 2)]
        pltpu.make_async_copy(buf, buf, sem_vl.at[g]).wait()

    def issue_wq(lo, hi):
        def body(k, c):
            for reg in range(4):
                r = pl.multiple_of(reg * 128 + (k // 4) * 8, 8)
                cc = pl.multiple_of((k % 4) * 1024, 1024)
                for a, src in enumerate((bwq, awq)):
                    pltpu.make_async_copy(src.at[pl.ds(r, 8), pl.ds(cc, 1024)],
                                          wqbuf.at[a, pl.ds(r, 8), pl.ds(cc, 1024)], sem_w.at[a]).start(priority=a)
            return c
        lax.fori_loop(lo, hi, body, 0)

    def issue_wo(lo, hi):
        def body(k, c):
            for reg in range(4):
                r = pl.multiple_of(reg * 1024 + k * 16, 16)
                for a, src in enumerate((bwo, awo)):
                    pltpu.make_async_copy(src.at[pl.ds(r, 16)], wobuf.at[a, pl.ds(r, 16)],
                                          sem_w.at[2 + a]).start(priority=a)
            return c
        lax.fori_loop(lo, hi, body, 0)

    def wait_wq(a):
        pltpu.make_async_copy(wqbuf.at[a], wqbuf.at[a], sem_w.at[a]).wait()

    def wait_wo(a):
        pltpu.make_async_copy(wobuf.at[a], wobuf.at[a], sem_w.at[2 + a]).wait()

    row8 = lax.broadcasted_iota(jnp.int32, (8, DH), 0)
    row8d = lax.broadcasted_iota(jnp.int32, (8, D), 0)

    def q_index(kind, t):
        b, h0, _ = coords(kind, t)
        return b * HG + h0 // G

    def load_q(kind, t):
        ph = 0 if kind == 'B' else 1
        base = q_index(kind, t)
        return [qbuf[ph, base + p].astype(bf16) for p in range(4 if kind == 'B' else 1)]

    def qk_head(kind, qs, t, i, S):
        p = i // 2 if kind == 'B' else 0
        s = lax.dot_general(qs[p], kvbuf[0, t % NS, i], (((1,), (1,)), ((), ())), preferred_element_type=f32)
        if S[p] is None:
            S[p] = s
        else:
            rr = lax.broadcasted_iota(jnp.int32, (8, R), 0)
            valid = (rr // 4 == i % 2) if kind == 'B' else (rr == i)
            S[p] = jnp.where(valid, s, S[p])

    def softmax_update(S, first):
        for p in range(len(S)):
            m_old = jnp.where(first, -jnp.inf, m_ref[p])
            l_old = jnp.where(first, 0.0, l_ref[p])
            m_new = jnp.maximum(m_old, jnp.max(S[p], axis=1, keepdims=True))
            alpha = jnp.exp((m_old - m_new) * SCALE)
            pr = jnp.exp((S[p] - m_new[:, 0:1]) * SCALE)
            lsum = pr[:, 0:128]
            for c in range(1, R // 128):
                lsum = lsum + pr[:, c * 128:(c + 1) * 128]
            l_ref[p] = alpha * l_old + lsum
            m_ref[p] = m_new
            a_ref[p] = alpha
            p_ref[p] = pr.astype(bf16)

    def pv_head(kind, P, t, i, PV):
        p = i // 2 if kind == 'B' else 0
        o = jnp.dot(P[p], kvbuf[1, t % NS, i], preferred_element_type=f32)
        if PV[p] is None:
            PV[p] = o
        else:
            valid = (row8 // 4 == i % 2) if kind == 'B' else (row8 == i)
            PV[p] = jnp.where(valid, o, PV[p])

    def project(ph, o, head0):
        ob = o.astype(bf16)
        out = None
        for r in range(G):
            hrow = pl.multiple_of((head0 + r) * DH, DH)
            y = jnp.dot(ob, wobuf[ph, pl.ds(hrow, DH), :], preferred_element_type=f32)
            out = y if out is None else jnp.where(row8d == r, y, out)
        return out

    def step(pv, qk, plan, t, pos=None, late_v=False):
        pos = POS if pos is None else pos

        def issue_at(p):
            for g, thunk in enumerate(plan):
                if pos[g] == p:
                    thunk()

        NP = 4 if pv == 'B' else 1
        P = [p_ref[p] for p in range(NP)]
        alphas = [a_ref[p] for p in range(NP)]
        l_cur = [l_ref[p] for p in range(NP)]
        if qk is not None:
            qs = load_q(qk, t + 1)
            wait_k(t + 1)
        if not late_v:
            wait_v(t)
        if qk is not None:
            S = [None] * (4 if qk == 'B' else 1)
            for i in range(G):
                issue_at(i)
                qk_head(qk, qs, t + 1, i, S)
        if late_v:
            with scope("lv_sm"):
                softmax_update(S, (t + 1) % NBLK == 0)
            with scope("lv_wait"):
                wait_v(t)
        PV = [None] * NP
        for i in range(G):
            issue_at(8 + i)
            pv_head(pv, P, t, i, PV)
        if qk is not None and not late_v:
            softmax_update(S, (t + 1) % NBLK == 0)
        first = t % NBLK == 0
        for p in range(NP):
            acc_ref[p] = jnp.where(first, PV[p], alphas[p] * acc_ref[p] + PV[p])
        issue_at(16)

        @pl.when(t % NBLK == NBLK - 1)
        def _():
            b, h0, _ = coords(pv, t)
            tot = None
            for p in range(NP):
                l = jnp.sum(l_cur[p], axis=1, keepdims=True)
                y = project(0 if pv == 'B' else 1, acc_ref[p] / l, h0 + 8 * p)
                tot = y if tot is None else tot + y
            row = jnp.sum(tot, axis=0, keepdims=True)
            ph = 0 if pv == 'B' else 1
            oacc[ph] = oacc[ph] + jnp.where(row8d == b, jnp.broadcast_to(row, (8, D)), 0.0)

    with scope("p_wq"):
        cx = pltpu.make_async_copy(x_hbm, xbuf, sem_small.at[0])
        cg = pltpu.make_async_copy(gw_hbm, gwbuf, sem_small.at[1])
        cx.start(); cg.start()
        issue_wq(0, 64)
        issue_wo(0, 16)

    with scope("p_x"):
        cx.wait(); cg.wait()
        xf = xbuf[...].astype(f32)
        x8 = jnp.zeros((8, D), f32)
        for b in range(B):
            x8 = jnp.where(row8d == b, jnp.broadcast_to(xf[b:b+1], (8, D)), x8)
        gw = gwbuf[...].astype(f32).reshape(1, D)
        gate = jax.nn.sigmoid(jnp.sum(x8 * gw, axis=-1, keepdims=True))
        x32 = jnp.concatenate([jnp.broadcast_to(xf[b:b+1], (8, D)) for b in range(B)], axis=0).astype(bf16)
        for ref in (m_ref, l_ref, a_ref, acc_ref, oacc):
            ref[...] = jnp.zeros(ref.shape, f32)

    def compute_q(a, hg):
        res = jnp.dot(x32, wqbuf[a, :, hg * G * DH:(hg + 1) * G * DH], preferred_element_type=f32)
        for b in range(B):
            q = res[8 * b:8 * b + 8, 0:DH]
            for r in range(1, G):
                q = jnp.where(row8 == r, res[8 * b:8 * b + 8, r * DH:(r + 1) * DH], q)
            qbuf[a, b * HG + hg] = q

    with scope("p_q"):
        wait_wq(0)
        wait_wq(1)
        for n in range(8):
            compute_q(n // HG, n % HG)
            issue_wo(16 + 6 * n, 16 + 6 * (n + 1))
    with scope("p_kv"):
        for thunk in plan_only(0, 'B', 0) + plan_pair('B', 1, 'B', 0) + plan_pair('B', 2, 'B', 1):
            thunk()
    with scope("p_qk0"):
        qs = load_q('B', 0)
        wait_k(0)
        S = [None] * 4
        for i in range(G):
            qk_head('B', qs, 0, i, S)
        softmax_update(S, True)
        wait_wo(0)
        wait_wo(1)

    def loop(pv, qk, kk, kv, lo, hi):
        def body(t, c):
            with scope("step"):
                step(pv, qk, plan_pair(kk, t + 3, kv, t + 2), t)
            return c
        lax.fori_loop(lo, hi, body, 0)

    def single(name, pv, qk, plan, t, pos=None, late_v=False):
        with scope(name):
            step(pv, qk, plan, t, pos, late_v)

    loop('B', 'B', 'B', 'B', 0, T_B - 3)
    t = T_B - 3
    single("s61", 'B', 'B', plan_pair('A', t + 3, 'B', t + 2), t)
    single("s62", 'B', 'B', plan_pair('A', t + 4, 'A', t + 3), t + 1)
    single("s63", 'B', 'A', plan_pair('A', t + 5, 'A', t + 4), t + 2)
    loop('A', 'A', 'A', 'A', T_B, T - 4)
    single("sT4", 'A', 'A', plan_only(0, 'A', T - 1) + plan_only(1, 'A', T - 2), T - 4)
    single("sT3", 'A', 'A', plan_vlast(T - 1), T - 3, pos=[8, 10, 12, 14])
    single("sT2", 'A', 'A', [], T - 2, late_v=True)

    t = T - 1
    b, h0, _ = coords('A', t)
    with scope("t_pre"):
        P = p_ref[0]
        rl = 1.0 / jnp.sum(l_ref[0], axis=1, keepdims=True)
        prev = a_ref[0] * acc_ref[0]
    tot = None
    for g in range(G // 2):
        with scope(f"t_pv{g}"):
            with scope(f"t_w{g}"):
                wait_vl(t, g)
            for i in (2 * g, 2 * g + 1):
                o = (prev + jnp.dot(P, kvbuf[1, t % NS, i], preferred_element_type=f32)) * rl
                hrow = (h0 + i) * DH
                y = jnp.dot(o.astype(bf16), wobuf[1, hrow:hrow + DH, :], preferred_element_type=f32)
                tot = y if tot is None else jnp.where(row8d == i, y, tot)
    with scope("t_fin"):
        row = jnp.sum(tot, axis=0, keepdims=True)
        outa = oacc[1] + jnp.where(row8d == b, jnp.broadcast_to(row, (8, D)), 0.0)
        res = gate * outa + (1.0 - gate) * oacc[0]
        outbuf[...] = res[0:B].astype(bf16)
    with scope("outdma"):
        co = pltpu.make_async_copy(outbuf, out_hbm, sem_small.at[2])
        co.start()
        co.wait()


@jax.jit
def pallas_gated_mix__mha_block_cached__gqa_block_cached__decode_kernel(A_x, A_k_cache, A_v_cache, A_wq, A_wo, B_x, B_k_cache, B_v_cache, B_wq, B_wo, gate_w):
    bf16 = jnp.bfloat16
    f32 = jnp.float32
    any_spec = pl.BlockSpec(memory_space=pl.ANY)
    out = pl.pallas_call(
        kernel,
        in_specs=[any_spec] * 10,
        out_specs=any_spec,
        out_shape=jax.ShapeDtypeStruct((B, D), bf16),
        scratch_shapes=[
            pltpu.VMEM((B, D), bf16),
            pltpu.VMEM((D,), bf16),
            pltpu.VMEM((2, D, H * DH), bf16),
            pltpu.VMEM((2, H * DH, D), bf16),
            pltpu.VMEM((2, NS, G, R, DH), bf16),
            pltpu.VMEM((2, B * HG, 8, DH), f32),
            pltpu.VMEM((4, 8, 128), f32),
            pltpu.VMEM((4, 8, 128), f32),
            pltpu.VMEM((4, 8, 128), f32),
            pltpu.VMEM((4, 8, R), bf16),
            pltpu.VMEM((4, 8, DH), f32),
            pltpu.VMEM((2, 8, D), f32),
            pltpu.VMEM((B, D), bf16),
            pltpu.SemaphoreType.DMA((3,)),
            pltpu.SemaphoreType.DMA((4,)),
            pltpu.SemaphoreType.DMA((NS,)),
            pltpu.SemaphoreType.DMA((NS,)),
            pltpu.SemaphoreType.DMA((G // 2,)),
        ],
        compiler_params=pltpu.CompilerParams(vmem_limit_bytes=100 * 1024 * 1024, disable_bounds_checks=bool(DBC)),
    )(A_x.reshape(B, D), A_k_cache, A_v_cache, A_wq, A_wo, B_k_cache, B_v_cache, B_wq, B_wo, gate_w)
    return out.reshape(B, 1, D)
```

```python
import functools

import jax
import jax.numpy as jnp
from jax import lax
from jax.experimental import pallas as pl
from jax.experimental.pallas import tpu as pltpu

B, D, H, HKV, SK, DH = 4, 512, 32, 8, 8192, 128
G = 8
R = 512
SR = 16
C = 64
NS = 3
NBLK = SK // R
NQ = R // SR
NGRP = 8
HG = H // G
T_B = B * NBLK
T_A = B * HG * NBLK
T = T_A + T_B
SCALE = DH ** -0.5
POS = (0, 2, 4, 6, 8, 10, 12, 14)


def _kernel(x_hbm, ak, av, awq, awo, bk, bv, bwq, bwo, gw_hbm, out_hbm,
            xbuf, gwbuf, wqbuf, wobuf, kvbuf, qbuf, m_ref, l_ref, a_ref, p_ref, acc_ref, oacc, outbuf,
            sem_small, sem_w, sem_k, sem_v, sem_vl):
    f32 = jnp.float32
    bf16 = jnp.bfloat16

    def coords(kind, t):
        if kind == 'B':
            return t // NBLK, 0, t % NBLK
        g = (t - T_B) // NBLK
        return g // HG, (g % HG) * G, t % NBLK

    def start_kv(which, kind, t, q, prio):
        b, h0, j = coords(kind, t)
        src = ((bk, bv) if kind == 'B' else (ak, av))[which]
        sem = (sem_k, sem_v)[which]
        pltpu.make_async_copy(src.at[b, pl.ds(h0, G), pl.ds(j * R + q * SR, SR)],
                              kvbuf.at[which, t % NS, :, pl.ds(q * SR, SR)], sem.at[t % NS]).start(priority=prio)

    def plan_pair(kk, tk, kv, tv):
        def grp(g):
            for q in range(g * NQ // NGRP, (g + 1) * NQ // NGRP):
                start_kv(0, kk, tk, q, 0)
                start_kv(1, kv, tv, q, 1)
        return [functools.partial(grp, g) for g in range(NGRP)]

    def plan_only(which, kind, t):
        def grp(g):
            for q in range(g * NQ // 4, (g + 1) * NQ // 4):
                start_kv(which, kind, t, q, q % 2)
        return [functools.partial(grp, g) for g in range(4)]

    def plan_vlast(t):
        b, h0, j = coords('A', t)

        def grp(g):
            for cc in range(R // C):
                for i in (2 * g, 2 * g + 1):
                    pltpu.make_async_copy(av.at[b, h0 + i, pl.ds(j * R + cc * C, C)],
                                          kvbuf.at[1, t % NS, i, pl.ds(cc * C, C)], sem_vl.at[g]).start(priority=1)
        return [functools.partial(grp, g) for g in range(G // 2)]

    def wait_k(t):
        buf = kvbuf.at[0, t % NS]
        pltpu.make_async_copy(buf, buf, sem_k.at[t % NS]).wait()

    def wait_v(t):
        buf = kvbuf.at[1, t % NS]
        pltpu.make_async_copy(buf, buf, sem_v.at[t % NS]).wait()

    def wait_vl(t, g):
        buf = kvbuf.at[1, t % NS, pl.ds(2 * g, 2)]
        pltpu.make_async_copy(buf, buf, sem_vl.at[g]).wait()

    def issue_wq(lo, hi):
        def body(k, c):
            for reg in range(4):
                r = pl.multiple_of(reg * 128 + (k // 4) * 8, 8)
                cc = pl.multiple_of((k % 4) * 1024, 1024)
                for a, src in enumerate((bwq, awq)):
                    pltpu.make_async_copy(src.at[pl.ds(r, 8), pl.ds(cc, 1024)],
                                          wqbuf.at[a, pl.ds(r, 8), pl.ds(cc, 1024)], sem_w.at[a]).start(priority=a)
            return c
        lax.fori_loop(lo, hi, body, 0)

    def issue_wo(lo, hi):
        def body(k, c):
            for reg in range(4):
                r = pl.multiple_of(reg * 1024 + k * 16, 16)
                for a, src in enumerate((bwo, awo)):
                    pltpu.make_async_copy(src.at[pl.ds(r, 16)], wobuf.at[a, pl.ds(r, 16)],
                                          sem_w.at[2 + a]).start(priority=a)
            return c
        lax.fori_loop(lo, hi, body, 0)

    def wait_wq(a):
        pltpu.make_async_copy(wqbuf.at[a], wqbuf.at[a], sem_w.at[a]).wait()

    def wait_wo(a):
        pltpu.make_async_copy(wobuf.at[a], wobuf.at[a], sem_w.at[2 + a]).wait()

    row8 = lax.broadcasted_iota(jnp.int32, (8, DH), 0)
    row8d = lax.broadcasted_iota(jnp.int32, (8, D), 0)

    def load_q(kind, t):
        b, h0, _ = coords(kind, t)
        base = b * HG + h0 // G
        return [qbuf[0 if kind == 'B' else 1, base + p].astype(bf16) for p in range(4 if kind == 'B' else 1)]

    def qk_head(kind, qs, t, i, S):
        p = i // 2 if kind == 'B' else 0
        s = lax.dot_general(qs[p], kvbuf[0, t % NS, i], (((1,), (1,)), ((), ())), preferred_element_type=f32)
        if S[p] is None:
            S[p] = s
        else:
            rr = lax.broadcasted_iota(jnp.int32, (8, R), 0)
            valid = (rr // 4 == i % 2) if kind == 'B' else (rr == i)
            S[p] = jnp.where(valid, s, S[p])

    def softmax_update(S, first):
        for p in range(len(S)):
            m_old = jnp.where(first, -jnp.inf, m_ref[p])
            l_old = jnp.where(first, 0.0, l_ref[p])
            m_new = jnp.maximum(m_old, jnp.max(S[p], axis=1, keepdims=True))
            alpha = jnp.exp((m_old - m_new) * SCALE)
            pr = jnp.exp((S[p] - m_new[:, 0:1]) * SCALE)
            lsum = pr[:, 0:128]
            for c in range(1, R // 128):
                lsum = lsum + pr[:, c * 128:(c + 1) * 128]
            l_ref[p] = alpha * l_old + lsum
            m_ref[p] = m_new
            a_ref[p] = alpha
            p_ref[p] = pr.astype(bf16)

    def pv_head(kind, P, t, i, PV):
        p = i // 2 if kind == 'B' else 0
        o = jnp.dot(P[p], kvbuf[1, t % NS, i], preferred_element_type=f32)
        if PV[p] is None:
            PV[p] = o
        else:
            valid = (row8 // 4 == i % 2) if kind == 'B' else (row8 == i)
            PV[p] = jnp.where(valid, o, PV[p])

    def project(ph, o, head0):
        ob = o.astype(bf16)
        out = None
        for r in range(G):
            hrow = pl.multiple_of((head0 + r) * DH, DH)
            y = jnp.dot(ob, wobuf[ph, pl.ds(hrow, DH), :], preferred_element_type=f32)
            out = y if out is None else jnp.where(row8d == r, y, out)
        return out

    def step(pv, qk, plan, t, pos=POS, late_v=False):
        def issue_at(p):
            for g, thunk in enumerate(plan):
                if pos[g] == p:
                    thunk()

        NP = 4 if pv == 'B' else 1
        P = [p_ref[p] for p in range(NP)]
        alphas = [a_ref[p] for p in range(NP)]
        l_cur = [l_ref[p] for p in range(NP)]
        qs = load_q(qk, t + 1)
        wait_k(t + 1)
        if not late_v:
            wait_v(t)
        S = [None] * (4 if qk == 'B' else 1)
        for i in range(G):
            issue_at(i)
            qk_head(qk, qs, t + 1, i, S)
        if late_v:
            softmax_update(S, (t + 1) % NBLK == 0)
            wait_v(t)
        PV = [None] * NP
        for i in range(G):
            issue_at(8 + i)
            pv_head(pv, P, t, i, PV)
        if not late_v:
            softmax_update(S, (t + 1) % NBLK == 0)
        first = t % NBLK == 0
        for p in range(NP):
            acc_ref[p] = jnp.where(first, PV[p], alphas[p] * acc_ref[p] + PV[p])

        @pl.when(t % NBLK == NBLK - 1)
        def _():
            b, h0, _ = coords(pv, t)
            ph = 0 if pv == 'B' else 1
            tot = None
            for p in range(NP):
                l = jnp.sum(l_cur[p], axis=1, keepdims=True)
                y = project(ph, acc_ref[p] / l, h0 + 8 * p)
                tot = y if tot is None else tot + y
            row = jnp.sum(tot, axis=0, keepdims=True)
            oacc[ph] = oacc[ph] + jnp.where(row8d == b, jnp.broadcast_to(row, (8, D)), 0.0)

    cx = pltpu.make_async_copy(x_hbm, xbuf, sem_small.at[0])
    cg = pltpu.make_async_copy(gw_hbm, gwbuf, sem_small.at[1])
    cx.start()
    cg.start()
    issue_wq(0, 64)
    issue_wo(0, 16)

    cx.wait()
    cg.wait()
    xf = xbuf[...].astype(f32)
    x8 = jnp.zeros((8, D), f32)
    for b in range(B):
        x8 = jnp.where(row8d == b, jnp.broadcast_to(xf[b:b + 1], (8, D)), x8)
    gw = gwbuf[...].astype(f32).reshape(1, D)
    gate = jax.nn.sigmoid(jnp.sum(x8 * gw, axis=-1, keepdims=True))
    x32 = jnp.concatenate([jnp.broadcast_to(xf[b:b + 1], (8, D)) for b in range(B)], axis=0).astype(bf16)
    for ref in (m_ref, l_ref, a_ref, acc_ref, oacc):
        ref[...] = jnp.zeros(ref.shape, f32)

    def compute_q(a, hg):
        res = jnp.dot(x32, wqbuf[a, :, hg * G * DH:(hg + 1) * G * DH], preferred_element_type=f32)
        for b in range(B):
            q = res[8 * b:8 * b + 8, 0:DH]
            for r in range(1, G):
                q = jnp.where(row8 == r, res[8 * b:8 * b + 8, r * DH:(r + 1) * DH], q)
            qbuf[a, b * HG + hg] = q

    wait_wq(0)
    wait_wq(1)
    for n in range(2 * HG):
        compute_q(n // HG, n % HG)
        issue_wo(16 + 6 * n, 16 + 6 * (n + 1))
    for thunk in plan_only(0, 'B', 0) + plan_pair('B', 1, 'B', 0) + plan_pair('B', 2, 'B', 1):
        thunk()
    qs0 = load_q('B', 0)
    wait_k(0)
    S0 = [None] * 4
    for i in range(G):
        qk_head('B', qs0, 0, i, S0)
    softmax_update(S0, True)
    wait_wo(0)
    wait_wo(1)

    def loop(pv, qk, kk, kv, lo, hi):
        def body(t, c):
            step(pv, qk, plan_pair(kk, t + 3, kv, t + 2), t)
            return c
        lax.fori_loop(lo, hi, body, 0)

    loop('B', 'B', 'B', 'B', 0, T_B - 3)
    t = T_B - 3
    step('B', 'B', plan_pair('A', t + 3, 'B', t + 2), t)
    step('B', 'B', plan_pair('A', t + 4, 'A', t + 3), t + 1)
    step('B', 'A', plan_pair('A', t + 5, 'A', t + 4), t + 2)
    loop('A', 'A', 'A', 'A', T_B, T - 3)
    step('A', 'A', plan_vlast(T - 1), T - 3, pos=(8, 10, 12, 14))
    step('A', 'A', [], T - 2, late_v=True)

    t = T - 1
    b, h0, _ = coords('A', t)
    P = p_ref[0]
    rl = 1.0 / jnp.sum(l_ref[0], axis=1, keepdims=True)
    prev = a_ref[0] * acc_ref[0]
    tot = None
    for g in range(G // 2):
        wait_vl(t, g)
        for i in (2 * g, 2 * g + 1):
            o = (prev + jnp.dot(P, kvbuf[1, t % NS, i], preferred_element_type=f32)) * rl
            hrow = (h0 + i) * DH
            y = jnp.dot(o.astype(bf16), wobuf[1, hrow:hrow + DH, :], preferred_element_type=f32)
            tot = y if tot is None else jnp.where(row8d == i, y, tot)
    row = jnp.sum(tot, axis=0, keepdims=True)
    outa = oacc[1] + jnp.where(row8d == b, jnp.broadcast_to(row, (8, D)), 0.0)
    res = gate * outa + (1.0 - gate) * oacc[0]
    outbuf[...] = res[0:B].astype(bf16)
    co = pltpu.make_async_copy(outbuf, out_hbm, sem_small.at[2])
    co.start()
    co.wait()


@jax.jit
def pallas_gated_mix__mha_block_cached__gqa_block_cached__decode_kernel(A_x, A_k_cache, A_v_cache, A_wq, A_wo, B_x, B_k_cache, B_v_cache, B_wq, B_wo, gate_w):
    del B_x
    bf16 = jnp.bfloat16
    f32 = jnp.float32
    any_spec = pl.BlockSpec(memory_space=pl.ANY)
    out = pl.pallas_call(
        _kernel,
        in_specs=[any_spec] * 10,
        out_specs=any_spec,
        out_shape=jax.ShapeDtypeStruct((B, D), bf16),
        scratch_shapes=[
            pltpu.VMEM((B, D), bf16),
            pltpu.VMEM((D,), bf16),
            pltpu.VMEM((2, D, H * DH), bf16),
            pltpu.VMEM((2, H * DH, D), bf16),
            pltpu.VMEM((2, NS, G, R, DH), bf16),
            pltpu.VMEM((2, B * HG, 8, DH), f32),
            pltpu.VMEM((4, 8, 128), f32),
            pltpu.VMEM((4, 8, 128), f32),
            pltpu.VMEM((4, 8, 128), f32),
            pltpu.VMEM((4, 8, R), bf16),
            pltpu.VMEM((4, 8, DH), f32),
            pltpu.VMEM((2, 8, D), f32),
            pltpu.VMEM((B, D), bf16),
            pltpu.SemaphoreType.DMA((3,)),
            pltpu.SemaphoreType.DMA((4,)),
            pltpu.SemaphoreType.DMA((NS,)),
            pltpu.SemaphoreType.DMA((NS,)),
            pltpu.SemaphoreType.DMA((G // 2,)),
        ],
        compiler_params=pltpu.CompilerParams(vmem_limit_bytes=64 * 1024 * 1024),
    )(A_x.reshape(B, D), A_k_cache, A_v_cache, A_wq, A_wo, B_k_cache, B_v_cache, B_wq, B_wo, gate_w)
    return out.reshape(B, 1, D)
```
